```python
import os as _os
_os.environ.setdefault("JAX_PLATFORMS", "cpu")
import jax
import jax.numpy as jnp

def _softmax(x, axis=-1):
    return jax.nn.softmax(x, axis=axis)
def _gelu(x):
    return jax.nn.gelu(x, approximate=True)
def _silu(x):
    return jax.nn.silu(x)
def _sigmoid(x):
    return jax.nn.sigmoid(x)
def _layernorm(x, axis=-1, eps=1e-5):
    m = jnp.mean(x, axis=axis, keepdims=True)
    v = jnp.var(x, axis=axis, keepdims=True)
    return (x - m) / jnp.sqrt(v + eps)
def _scatter_add(tgt, idx, src, axis=0):
    return tgt.at[idx].add(src)
def _segment_sum(src, seg, n):
    return jax.ops.segment_sum(src, seg, n)
class _Rng:
    def __init__(self, key):
        self._k = key
    def _next(self):
        self._k, sub = jax.random.split(self._k)
        return sub
    def normal(self, shape):
        return jax.random.normal(self._next(), shape, dtype=jnp.bfloat16)
    def randint(self, lo, hi, shape):
        return jax.random.randint(self._next(), shape, lo, hi, dtype=jnp.int32)
    def uniform(self, shape, lo=0.0, hi=1.0):
        return jax.random.uniform(self._next(), shape, jnp.bfloat16, lo, hi)
    def permutation(self, n):
        return jax.random.permutation(self._next(), n)


kernel_name = 'recurrent_scan__softmax_full_mha__glu_gated_glu__prompt'

def setup_inputs():
    _rng = _Rng(jax.random.key(int.from_bytes(__import__("os").urandom(4), "little")))
    _w = (lambda a: (lambda t: t.astype(jnp.bfloat16) if jnp.issubdtype(t.dtype, jnp.floating) else t)(jnp.asarray(a)))
    def _A_setup():
        B, S, D = 1, 2048, 1024
        return {
            "x": _w((lambda *s: _rng.normal(s) * 0.05)(B, S, D)),
            "wqkv": _w((lambda *s: _rng.normal(s) * 0.05)(D, 3 * D)),
            "wo": _w((lambda *s: _rng.normal(s) * 0.05)(D, D)),
        }
    _A_in = _A_setup()

    def _B_setup():
        B, S, D, F = 1, 2048, 1024, 3584
        return {
            "x": _w((lambda *s: _rng.normal(s) * 0.05)(B, S, D)),
            "w_gate": _w((lambda *s: _rng.normal(s) * 0.05)(D, F)),
            "w_up": _w((lambda *s: _rng.normal(s) * 0.05)(D, F)),
            "w_down": _w((lambda *s: _rng.normal(s) * 0.05)(F, D)),
        }
    _B_in = _B_setup()

    return {
        "A_x": _A_in["x"],
        "A_wqkv": _A_in["wqkv"],
        "A_wo": _A_in["wo"],
        "B_x": _B_in["x"],
        "B_w_gate": _B_in["w_gate"],
        "B_w_up": _B_in["w_up"],
        "B_w_down": _B_in["w_down"],
    }

def reference(A_x, A_wqkv, A_wo, B_x, B_w_gate, B_w_up, B_w_down):
    def _A_ref(x, wqkv, wo):
        B, S, D = x.shape
        H = 32; Dh = D // H
        qkv = (lambda x, *d: x.transpose(*d))((x @ wqkv).reshape(B, S, 3, H, Dh), 2, 0, 3, 1, 4)
        q, k, v = qkv[0], qkv[1], qkv[2]
        scale = Dh ** -0.5
        scores = jnp.einsum("bhqd,bhkd->bhqk", q, k) * scale
        p = _softmax(scores, axis=-1)
        o = jnp.einsum("bhqk,bhkd->bhqd", p, v)
        return (lambda x, *d: x.transpose(*d))(o, 0, 2, 1, 3).reshape(B, S, D) @ wo

    def _B_ref(x, w_gate, w_up, w_down):
        g = jnp.einsum("bsd,df->bsf", x, w_gate)
        u = jnp.einsum("bsd,df->bsf", x, w_up)
        h = _sigmoid(g) * u
        return jnp.einsum("bsf,fd->bsd", h, w_down)

    x = A_x
    xn = _layernorm(x, axis=-1)
    s = _A_ref(xn, A_wqkv, A_wo)
    g = _silu(_B_ref(xn, B_w_gate, B_w_up, B_w_down))
    return x + s * g
```

```python
import jax
import jax.numpy as jnp
import numpy as np
from jax import lax
import jax.experimental.pallas as pl
import jax.experimental.pallas.tpu as pltpu

TOK_C = 1
F32 = jnp.float32
BF16 = jnp.bfloat16

SEQ, DIM, FFN = 2048, 1024, 3584
HEAD_DIM = 32
EPS = 1e-5
Q_SCALE = float(HEAD_DIM ** -0.5 * np.log2(np.e))

NP = 49
ROWS = 128
TOK = 4 * ROWS
NT = SEQ // TOK
NG = DIM // 128
NF = FFN // 512
CK = 128
HALF = ROWS // 2

LHS_SUMS = (
    ((1, 0, 0), (1, 1, 1)), ((1, 1, 0), (1, 1, 1)), ((1, 0, 0),), ((1, 1, 1),),
    ((1, 0, 0), (1, 0, 1)), ((1, 1, 0), (-1, 0, 0)), ((1, 0, 1), (-1, 1, 1)),
)
RHS_SUMS = (
    ((1, 0, 0), (1, 1, 1)), ((1, 0, 0),), ((1, 0, 1), (-1, 1, 1)),
    ((1, 1, 0), (-1, 0, 0)), ((1, 1, 1),), ((1, 0, 0), (1, 0, 1)),
    ((1, 1, 0), (1, 1, 1)),
)


def _signed_sum(terms, get):
    acc = None
    for sign, r, c in terms:
        v = get(r, c)
        acc = v if acc is None else (acc + v if sign > 0 else acc - v)
    return acc


def _operands(sums, i, block):
    outer = {
        (r, c): _signed_sum(sums[i], lambda p, q: block(2 * p + r, 2 * q + c))
        for r in range(2) for c in range(2)
    }
    return [_signed_sum(sums[j], lambda p, q: outer[p, q]) for j in range(7)]


def _recombine2(m):
    return {
        (0, 0): m[0] + m[3] - m[4] + m[6], (0, 1): m[2] + m[4],
        (1, 0): m[1] + m[3], (1, 1): m[0] - m[1] + m[2] + m[5],
    }


def _recombine4(product, fence):
    inner = []
    for i in range(7):
        fence()
        inner.append(_recombine2([product(7 * i + j) for j in range(7)]))
        yield (inner[i][0, 0], inner[i][1, 1]) if TOK_C else ()
    out = {}
    for r in range(2):
        for c in range(2):
            for (p, q), v in _recombine2([t[r, c] for t in inner]).items():
                out[2 * p + r, 2 * q + c] = v
    return out


def _times_sigmoid(v, g):
    hv = 0.5 * v
    return hv * jnp.tanh(0.5 * g) + hv


class _Timeline:
    def __init__(self, never):
        self.never = never
        self.items = []
        self.pending = []
        self.latest = None

    def add(self, stage, start, end=None):
        steps, gen = stage
        end = start + 1 if end is None else end
        for k in range(steps + 1):
            when = start + (end - start) * min(k + 0.5, steps - 0.5) / steps
            self.items.append((when, len(self.items), gen, k == steps))

    def call(self, when, *fns):
        def gen():
            for fn in fns:
                fn()
            yield ()
        self.add((1, gen()), when, when)

    def fence(self, buf, index):
        if self.latest is not None:
            buf[index, :8, :128] = self.latest
            self.latest = None

    def tie(self, value):
        self.latest = value[:8, :128]
        if not self.pending:
            return value
        token = self.pending[0][:8, :128]
        for v in self.pending[1:]:
            token = jnp.maximum(token, v[:8, :128])
        self.pending = []
        head = jnp.where(self.never, token, value[:8, :128])
        head = jnp.concatenate([head, value[:8, 128:]], axis=1)
        return jnp.concatenate([head, value[8:]], axis=0)

    def emit(self):
        for _, _, gen, done in sorted(self.items, key=lambda e: e[:2]):
            tokens = next(gen, None)
            assert (tokens is None) == done
            self.pending += tokens or ()


def _stage(steps):
    def wrap(fn):
        return lambda *args: (steps, fn(*args))
    return wrap


def _kernel(x_hbm, wqkv_hbm, wo_hbm, wg_hbm, wu_hbm, wd_hbm, out_hbm,
            x_v, w_v, wd_v, a_v, b_v, bd_v, m0_v, m1_v, o_v, ot_v, l_v, mx_v,
            idx_s, x_sem, w_sem, wd_sem, out_sem):
    m_v = (m0_v, m1_v)
    spare = lax.fori_loop(0, 2, lambda i, c: c * c + 2 * i, 2) + NP - 18

    def x_copy(t):
        return pltpu.make_async_copy(x_hbm.at[t], x_v.at[t], x_sem.at[t])

    def out_copy(t, half):
        rows = pl.ds(half * HALF, HALF)
        return pltpu.make_async_copy(
            x_v.at[t, :, rows], out_hbm.at[t, :, rows], out_sem.at[2 * t + half])

    def wqkv_copy(part, slot):
        return pltpu.make_async_copy(
            wqkv_hbm.at[:, pl.ds(part * DIM, DIM)], w_v.at[slot], w_sem.at[slot, 0])

    def wo_copy(slot):
        return pltpu.make_async_copy(wo_hbm, w_v.at[slot], w_sem.at[slot, 0])

    def glu_copies(g):
        slot = (g + 1) % 2
        cols = pl.ds(pl.multiple_of(g * 512, 512), 512)
        return [
            pltpu.make_async_copy(
                w.at[:, cols], w_v.at[slot, :, pl.ds(512 * n, 512)], w_sem.at[slot, n])
            for n, w in enumerate((wg_hbm, wu_hbm))
        ]

    def wd_copy(g):
        rows = pl.ds(pl.multiple_of(g * 512, 512), 512)
        return pltpu.make_async_copy(wd_hbm.at[rows], wd_v.at[g % 2], wd_sem.at[g % 2])

    def timeline():
        v = x_v[0, 0, :8, :128].astype(F32)
        return _Timeline(v * v < 0)

    @_stage(ROWS // 8 * 11)
    def layernorm_operands(t):
        for r0 in range(0, ROWS, 8):
            xn = []
            for a in range(4):
                x = x_v[t, a, r0:r0 + 8, :].astype(F32)
                xc = x - jnp.mean(x, axis=-1, keepdims=True)
                var = jnp.mean(xc * xc, axis=-1, keepdims=True)
                xn.append(xc * lax.rsqrt(var + EPS))
                yield xn[-1:]
            for i in range(7):
                ops = _operands(LHS_SUMS, i, lambda a, k: xn[a][:, 256 * k:256 * (k + 1)])
                for j, v in enumerate(ops):
                    a_v[t, 7 * i + j, r0:r0 + 8, :] = v.astype(BF16)
                yield ops[5:]

    @_stage(ROWS // 8 * 7)
    def attention_out_operands(t):
        for i in range(7):
            for r0 in range(0, ROWS, 8):
                def block(a, k):
                    rows = slice(ROWS * a + r0, ROWS * a + r0 + 8)
                    return jnp.concatenate(
                        [o_v[t, 2 * k, rows, :], o_v[t, 2 * k + 1, rows, :]], axis=1)
                ops = _operands(LHS_SUMS, i, block)
                for j, v in enumerate(ops):
                    a_v[t, 7 * i + j, r0:r0 + 8, :] = v.astype(BF16)
                yield ops[5:] + [v[:, 128:] for v in ops[5:]]

    @_stage(256 // 8)
    def weight_operands(slot, i):
        for r0 in range(0, 256, 8):
            def block(k, c):
                return w_v[slot, 256 * k + r0:256 * k + r0 + 8,
                           256 * c:256 * (c + 1)].astype(F32)
            ops = _operands(RHS_SUMS, i, block)
            for j, v in enumerate(ops):
                b_v[7 * i + j, r0:r0 + 8, :] = v.astype(BF16)
            yield ops[5:]

    def add_weight_operands(tl, slot, first_use):
        for i in range(7):
            start = first_use - 0.8 + i * 1.5 / 7
            tl.add(weight_operands(slot, i), start, start + 1.5 / 7)

    @_stage(128 // 8 * 7)
    def down_operands(g):
        for i in range(7):
            for r0 in range(0, 128, 8):
                def block(k, c):
                    return wd_v[g % 2, 128 * k + r0:128 * k + r0 + 8,
                                256 * c:256 * (c + 1)].astype(F32)
                ops = _operands(RHS_SUMS, i, block)
                for j, v in enumerate(ops):
                    bd_v[g, 7 * i + j, r0:r0 + 8, :] = v.astype(BF16)
                yield ops[5:]

    @_stage(NP * ROWS // 16)
    def products(tl, t):
        for r in range(NP):
            m = jnp.dot(a_v[t, r], b_v[r], preferred_element_type=F32)
            for r0 in range(0, ROWS, 16):
                m_v[t % 2][r, r0:r0 + 16] = tl.tie(m[r0:r0 + 16])
                yield ()

    def blocks(tl, buf, r0, p):
        return _recombine4(lambda r: buf[r, r0:r0 + 8, 128 * p:128 * (p + 1)],
                           lambda: tl.fence(buf, spare))

    @_stage(4)
    def normalize(item):
        for a in range(4):
            cols = slice(ROWS * a, ROWS * (a + 1))
            o = jnp.concatenate([
                ot_v[j, :, cols] / jnp.sum(l_v[j, :, cols], axis=0, keepdims=True)
                for j in range(4)], axis=0).T
            o_v[item // NG, item % NG, cols, :] = o
            yield [o]

    def attention(k_v, qt_v, vt_v, s_v):
        @_stage(ROWS // 8 * 2 * 7)
        def recombine_k(tl, t):
            for r0 in range(0, ROWS, 8):
                for p in range(2):
                    out = yield from blocks(tl, m_v[t % 2], r0, p)
                    for (a, c), v in out.items():
                        row = TOK * t + ROWS * a + r0
                        k_v[2 * c + p, row:row + 8, :] = v.astype(BF16)

        @_stage(ROWS // 8 * 2 * 7)
        def recombine_qv(tl, t, is_q):
            for r0 in range(0, ROWS, 8):
                for p in range(2):
                    out = yield from blocks(tl, m_v[t % 2], r0, p)
                    for (a, c), v in out.items():
                        row = ROWS * a + r0
                        o_v[t, 2 * c + p, row:row + 8, :] = v * Q_SCALE if is_q else v

        @_stage(NG * 4)
        def transpose_qv(t, is_q):
            for g in range(NG):
                for a in range(4):
                    v = o_v[t, g, ROWS * a:ROWS * (a + 1), :].T
                    if is_q:
                        qt_v[t, g, :, ROWS * a:ROWS * (a + 1)] = v.astype(BF16)
                    else:
                        col = TOK * t + ROWS * a
                        vt_v[g, :, col:col + ROWS] = v.astype(BF16)
                    yield [v]

        @_stage(4 * SEQ // CK)
        def tile(tl, cur, nxt):
            for j in range(4):
                m = l = o = None
                if cur is not None:
                    row_max = mx_v[j]
                if nxt is not None:
                    q = qt_v[nxt // NG, nxt % NG, HEAD_DIM * j:HEAD_DIM * (j + 1), :]
                    if j:
                        q = jnp.concatenate(
                            [jnp.zeros((HEAD_DIM * j, TOK), BF16), q], axis=0)
                for c in range(SEQ // CK):
                    keys = slice(CK * c, CK * (c + 1))
                    if cur is not None:
                        s_old = s_v[j, keys, :]
                    if nxt is not None:
                        s = jnp.dot(k_v[nxt % NG, keys, :HEAD_DIM * (j + 1)], q,
                                    preferred_element_type=F32)
                        s_v[j, keys, :] = tl.tie(s)
                        for r in range(0, CK, 8):
                            m = s[r:r + 8] if m is None else jnp.maximum(m, s[r:r + 8])
                    if cur is not None:
                        p = [jnp.exp2(s_old[r:r + 8] - row_max) for r in range(0, CK, 8)]
                        for v in p:
                            l = v if l is None else l + v
                        pv = jnp.dot(
                            vt_v[cur % NG, HEAD_DIM * j:HEAD_DIM * (j + 1), keys],
                            jnp.concatenate(p, axis=0).astype(BF16),
                            preferred_element_type=F32)
                        o = pv if o is None else o + pv
                    yield ()
                if nxt is not None:
                    mx_v[j] = jnp.broadcast_to(jnp.max(m, axis=0, keepdims=True), m.shape)
                if cur is not None:
                    l_v[j] = l
                    ot_v[j] = o

        x_copy(0).start()
        wqkv_copy(1, 0).start()
        for t in range(1, NT):
            x_copy(t).start()
        wqkv_copy(0, 1).start()
        wd_copy(0).start()
        ot_v[...] = jnp.zeros_like(ot_v)
        l_v[...] = jnp.ones_like(l_v)

        x_copy(0).wait()
        tl = timeline()
        for t in range(NT):
            if t: tl.call(t - 1, x_copy(t).wait)
            tl.add(layernorm_operands(t), t - 1, t - (0.2 if t == 0 else 0.05))
        tl.call(-0.2, wqkv_copy(1, 0).wait)
        for i in range(7):
            tl.add(weight_operands(0, i), (i - 1.2) / 7.5, (i - 0.2) / 7.5)
        tl.call(1, wqkv_copy(2, 0).start)
        tl.call(2, wqkv_copy(0, 1).wait)
        add_weight_operands(tl, 1, NT)
        tl.call(NT + 1, *[c.start for c in glu_copies(0)], wqkv_copy(2, 0).wait)
        add_weight_operands(tl, 0, 2 * NT)
        tl.call(2 * NT + 1, *[c.start for c in glu_copies(1)],
                *[c.wait for c in glu_copies(0)])
        add_weight_operands(tl, 1, 3 * NT)
        for t in range(NT):
            for n in range(3):
                tl.add(products(tl, t), n * NT + t)
            tl.add(recombine_k(tl, t), t + 1)
            tl.add(recombine_qv(tl, t, True), NT + t + 1)
            tl.add(transpose_qv(t, True), NT + t + 2)
            last = t == NT - 1
            tl.add(recombine_qv(tl, t, False), 2 * NT + t + 1, 2 * NT + t + (1.6 if last else 2))
            tl.add(transpose_qv(t, False), 2 * NT + t + (1.6 if last else 2),
                   min(2 * NT + t + 3, 3 * NT + 0.95))
        tl.add(tile(tl, None, 0), 3 * NT)
        tl.emit()

        n_items = NT * NG

        def body(i, carry):
            tl = timeline()
            tl.add(normalize(jnp.maximum(i - 1, 0)), 0, 0.2)
            tl.add(tile(tl, i, i + 1), 0)
            tl.emit()
            return carry

        lax.fori_loop(0, n_items - 1, body, 0)

        tl = timeline()
        tl.add(products(tl, 0), 0)
        tl.add(normalize(n_items - 2), 0, 0.2)
        tl.add(tile(tl, n_items - 1, None), 0.01, 1.01)
        tl.emit()

    pl.run_scoped(
        attention,
        pltpu.VMEM((NG, SEQ, 128), BF16),
        pltpu.VMEM((NT, NG, 128, TOK), BF16),
        pltpu.VMEM((NG, 128, SEQ), BF16),
        pltpu.VMEM((4, SEQ, TOK), F32),
    )

    def glu(h_v):
        @_stage(ROWS // 8 * 21)
        def recombine_gated(tl, g, t):
            for r0 in range(0, ROWS, 8):
                h = {}
                for p in range(2):
                    out = yield from blocks(tl, m_v[t % 2], r0, p)
                    for a in range(4):
                        for c in range(2):
                            h[a, 2 * c + p] = _times_sigmoid(out[a, c + 2], out[a, c])
                for i in range(7):
                    ops = _operands(LHS_SUMS, i, lambda a, k: h[a, k])
                    h_v[t, g, i, r0:r0 + 8, :] = jnp.concatenate(ops, axis=1).astype(BF16)
                    yield ops[5:]

        @_stage(NP * 2 * HALF // 16)
        def out_products(tl, t, half):
            rows = slice(HALF * half, HALF * (half + 1))
            for r in range(NP):
                i, j = divmod(r, 7)
                y = None
                for g in range(NF):
                    d = jnp.dot(h_v[t, g, i, rows, 128 * j:128 * (j + 1)], bd_v[g, r],
                                preferred_element_type=F32)
                    y = d if y is None else y + tl.tie(d)
                    yield ()
                m_v[half][r, :HALF] = y
                m_v[half][r, HALF:] = tl.tie(
                    jnp.dot(a_v[t, r, rows], b_v[r], preferred_element_type=F32))
                yield ()

        @_stage(HALF // 8 * 2 * 15)
        def recombine_out(tl, t, half):
            for r0 in range(0, HALF, 8):
                for p in range(2):
                    y = yield from blocks(tl, m_v[half], r0, p)
                    gate = {k: _times_sigmoid(v, v) for k, v in y.items()}
                    s = yield from blocks(tl, m_v[half], HALF + r0, p)
                    rows = slice(HALF * half + r0, HALF * half + r0 + 8)
                    outs = []
                    for (a, c), v in s.items():
                        cols = slice(256 * c + 128 * p, 256 * c + 128 * (p + 1))
                        outs.append(x_v[t, a, rows, cols].astype(F32) + v * gate[a, c])
                        x_v[t, a, rows, cols] = outs[-1].astype(BF16)
                    yield outs

        def group(g):
            tl = timeline()
            for t in range(1, NT):
                tl.add(products(tl, t), t)
            for t in range(NT):
                tl.add(recombine_gated(tl, g, t), t + 1, t + 1.98)
            tl.add(down_operands(g), 1, 3.2)
            add_weight_operands(tl, g % 2, NT)
            return tl

        def body(g, carry):
            wd_copy(g + 1).start()

            @pl.when(g + 2 < NF)
            def _():
                for c in glu_copies(g + 2):
                    c.start()

            @pl.when(g + 2 == NF)
            def _():
                wo_copy((NF + 1) % 2).start()

            wd_copy(g).wait()
            for c in glu_copies(g + 1):
                c.wait()
            tl = group(g)
            tl.add(products(tl, 0), NT)
            tl.emit()
            return carry

        lax.fori_loop(0, NF - 1, body, 0)

        wd_copy(NF - 1).wait()
        wo_copy((NF + 1) % 2).wait()
        tl = group(NF - 1)
        tl.add(normalize(NT * NG - 1), 1)
        for t in range(NT):
            tl.add(attention_out_operands(t), t + 1, t + 1.98)
        tl.add(out_products(tl, 0, 0), NT)
        tl.emit()

        def out_body(t, carry):
            tl = timeline()
            tl.add(out_products(tl, t, 1), 0)
            tl.add(recombine_out(tl, t, 0), 0, 0.98)
            tl.add(out_products(tl, t + 1, 0), 1)
            tl.add(recombine_out(tl, t, 1), 1, 1.98)
            tl.emit()
            out_copy(t, 0).start()
            out_copy(t, 1).start()
            return carry

        lax.fori_loop(0, NT - 1, out_body, 0)

        tl = timeline()
        tl.add(out_products(tl, NT - 1, 1), 0)
        tl.add(recombine_out(tl, NT - 1, 0), 0, 0.9)
        tl.call(1, out_copy(NT - 1, 0).start)
        tl.add(recombine_out(tl, NT - 1, 1), 1)
        tl.call(2, out_copy(NT - 1, 1).start)
        tl.emit()
        for t in range(NT):
            for half in range(2):
                out_copy(t, half).wait()

    pl.run_scoped(glu, pltpu.VMEM((NT, NF, 7, ROWS, 7 * 128), BF16))


@jax.jit
def pallas_recurrent_scan__softmax_full_mha__glu_gated_glu__prompt_kernel(
    A_x: jax.Array,
    A_wqkv: jax.Array,
    A_wo: jax.Array,
    B_x: jax.Array,
    B_w_gate: jax.Array,
    B_w_up: jax.Array,
    B_w_down: jax.Array,
):
    del B_x
    assert A_x.shape == (1, SEQ, DIM) and B_w_gate.shape == (DIM, FFN)
    tiled = (NT, 4, ROWS, DIM)
    out = pl.pallas_call(
        _kernel,
        out_shape=jax.ShapeDtypeStruct(tiled, BF16),
        in_specs=[pl.BlockSpec(memory_space=pl.ANY)] * 6,
        out_specs=pl.BlockSpec(memory_space=pl.ANY),
        scratch_shapes=[
            pltpu.VMEM(tiled, BF16),
            pltpu.VMEM((2, DIM, DIM), BF16),
            pltpu.VMEM((2, 512, DIM), BF16),
            pltpu.VMEM((NT, NP, ROWS, 256), BF16),
            pltpu.VMEM((NP, 256, 256), BF16),
            pltpu.VMEM((NF, NP, 128, 256), BF16),
            pltpu.VMEM((NP + 1, ROWS, 256), F32),
            pltpu.VMEM((NP + 1, ROWS, 256), F32),
            pltpu.VMEM((NT, NG, TOK, 128), F32),
            pltpu.VMEM((4, HEAD_DIM, TOK), F32),
            pltpu.VMEM((4, 8, TOK), F32),
            pltpu.VMEM((4, 8, TOK), F32),
            pltpu.SMEM((1,), jnp.int32),
            pltpu.SemaphoreType.DMA((NT,)),
            pltpu.SemaphoreType.DMA((2, 2)),
            pltpu.SemaphoreType.DMA((2,)),
            pltpu.SemaphoreType.DMA((2 * NT,)),
        ],
        compiler_params=pltpu.CompilerParams(vmem_limit_bytes=127 * 2**20),
        name="mha_glu",
    )(A_x.reshape(tiled), A_wqkv, A_wo, B_w_gate, B_w_up, B_w_down)
    return out.reshape(A_x.shape)
```

```python
import jax
import jax.numpy as jnp
import numpy as np
from jax import lax
import jax.experimental.pallas as pl
import jax.experimental.pallas.tpu as pltpu

F32 = jnp.float32
BF16 = jnp.bfloat16

SEQ, DIM, FFN = 2048, 1024, 3584
HEAD_DIM = 32
EPS = 1e-5
Q_SCALE = float(HEAD_DIM ** -0.5 * np.log2(np.e))

BLK = 128
PAD = 8
NR = SEQ // BLK
ND = DIM // BLK
TOK = 4 * BLK
GB = 2
STEPS = SEQ // TOK * ND // GB
LAG = 2

SIZES = {"x": SEQ * BLK, "hidden": 2 * SEQ * DIM, "qv": 2 * DIM * DIM, "gate0": DIM * DIM,
         "gate": DIM * (FFN - DIM), "up": DIM * FFN, "down": 2 * DIM * DIM}


def _dot(lhs, rhs):
    return lax.dot_general(lhs, rhs, (((1,), (0,)), ((), ())), precision=lax.Precision.DEFAULT,
                           preferred_element_type=F32)


def _total(values):
    acc = None
    for v in values:
        acc = v if acc is None else acc if v is None else acc + v
    return acc


def _sigmoid(v, scale=1.0):
    return 0.5 * jnp.tanh(0.5 * scale * v) + 0.5


def _silu(v):
    half = 0.5 * v
    return half * jnp.tanh(half) + half


def _block(n):
    return pl.ds(n * BLK if isinstance(n, int) else pl.multiple_of(n * BLK, BLK), BLK)


def _blocks(*counts):
    return pltpu.VMEM((*counts, BLK + PAD, BLK), F32)


def _unpadded(ref):
    return ref.at[..., :BLK, :]


def _pair_scratch(n):
    return [_blocks(n, ND), _blocks(n), _blocks(ND), _blocks(ND), _blocks(n)]


def _run(gen):
    for _ in gen:
        pass


class _Pair:
    def __init__(self, scratch, n, p, a, b, x, y, c_done, z_done, b_scale=None,
                 c_init=lambda i, k: None, z_init=lambda i, j: None):
        self.scratch, self.n, self.p = scratch, n, p
        self.a, self.b, self.x, self.y = a, b, x, y
        self.c_done, self.z_done = c_done, z_done
        self.c_init, self.z_init = c_init, z_init
        self.scaled = lambda v: v if b_scale is None else v * b_scale

    def row(self, tl, i, early=False):
        b_v, sum_b, sum_x, w_c, w_z = self.scratch
        n, p = self.n, self.p
        first = isinstance(i, int) and i == 0
        ready = not (first or early)
        y = [self.y(k, i).astype(F32) for k in range(p)]
        minus_y = -_total(y)
        c = {k: _total([w_c[k] if ready else None, self.c_init(i, k)]) for k in range(p)}
        wc, all_a = {}, []

        def right(e, at):
            if not isinstance(i, int) or i > e // 2:
                return b_v[at]
            b = self.scaled(self.b(*at).astype(F32))
            if i == e // 2:
                b_v[at] = b
            return b

        def add(cols, rows, patch, prod):
            for e in range(2):
                j, k = patch[3 * e]
                cols[k] = _total([cols.get(k), prod[e] + prod[e + 2]])
                rows[j] = _total([rows.get(j), prod[2 * e] + prod[2 * e + 1]])

        def sums(j, k):
            out = []
            if j is not None:
                out.append(self.scaled(_total(self.b(j, e).astype(F32) for e in range(p))))
                sum_b[j] = out[-1]
            if k is not None:
                out.append(_total(self.x(e, k) for e in range(n)))
                sum_x[k] = out[-1]
            return out

        def corrected(v, w, w_ref, at):
            if first:
                minus_w = -self.scaled(w[at])
                w_ref[at] = minus_w
                return v + minus_w
            return v + w_ref[at] if early else v

        for j4 in range(0, n, 4):
            a, wz = {j: self.a(i, j) for j in range(j4, j4 + 4)}, {}
            z = {j: _total([w_z[j] if ready else None, self.z_init(i, j)]) for j in a}
            for j0 in (j4, j4 + 2):
                for k0 in range(0, p, 2):
                    patch = [(j, k) for j in (j0, j0 + 1) for k in (k0, k0 + 1)]
                    pinned = [minus_y] if (j0, k0) == (2, 0) else []
                    if first:
                        last = j0 == n - 2
                        add(wc, wz, patch, tl.products(
                            [(self.x(*at), self.b(*at)) for at in patch],
                            sums(j0 + k0 // 2 if k0 < 4 else None, k0 if last else None)))
                        yield []
                        pinned += sums(None, k0 + 1 if last else None)
                    add(c, z, patch, tl.products(
                        [(a[j] + self.x(j, k), right(e, (j, k)) + y[k])
                         for e, (j, k) in enumerate(patch)], pinned))
                    yield []
            for j, v in zip(a, tl.products([(a[j], minus_y - sum_b[j]) for j in a])):
                self.z_done(i, j, corrected(v + z[j], wz, w_z, j))
            all_a += a.values()
            yield []
        minus_a = -_total(all_a)
        for k4 in range(0, p, 4):
            part = range(k4, k4 + 4)
            for k, v in zip(part, tl.products([(minus_a - sum_x[k], y[k]) for k in part])):
                self.c_done(i, k, corrected(v + c[k], wc, w_c, k))
            yield []

    def rows(self, tl, start, count):
        for n in range(count):
            _run(self.row(tl, start + n))

    def loop(self, timeline, start, loops, unroll):
        def body(step, carry):
            self.rows(timeline(), start + step * unroll, unroll)
            return carry
        lax.fori_loop(0, loops, body, 0)


class _Timeline:
    def __init__(self, never):
        self.never = never
        self.items = []
        self.pending = []
        self.latest = None

    def add(self, steps, gen, start=0.0, end=1.0):
        for k in range(steps):
            when = start + (end - start) * (k + 0.5) / steps
            self.items.append((when, len(self.items), gen))

    def fence(self, ref, *index):
        if self.latest is not None:
            ref[index + (slice(0, 128),)] = self.latest.astype(ref.dtype)
            self.latest = None

    def tie(self, value, row=0):
        self.latest = value[row:row + 8, :128]
        if not self.pending:
            return value
        head = lax.select(self.never, self.pending.pop(0)[:8, :128], self.latest)
        if value.shape[1] > 128:
            head = jnp.concatenate([head, value[row:row + 8, 128:]], axis=1)
        return jnp.concatenate(([value[:row]] if row else []) + [head, value[row + 8:]])

    def products(self, operands, pinned=()):
        out = [self.tie(_dot(*e), row) for e, row in zip(operands, (0, 64, 96, 32))]
        for e, v in enumerate(pinned):
            out[e] = lax.select(jnp.concatenate([self.never] * (BLK // 8)), v, out[e])
        return out

    def emit(self):
        for _, _, gen in sorted(self.items, key=lambda e: e[:2]):
            self.pending += next(gen)
        self.items, self.pending, self.latest = [], [], None


def _kernel(x_hbm, wqkv_hbm, wo_hbm, wg_hbm, wu_hbm, wd_hbm, out_hbm,
            in_sem, out_sem, x_v, wg_v, wu_v, wd_v, size_v, factor_v, *blocks):
    xn_v, o_v, h_v, *scratch = map(_unpadded, blocks)

    def timeline():
        v = x_v[0, :8, :128].astype(F32)
        return _Timeline(v * v < 0)

    def measure(name, slot, v):
        at = (list(SIZES).index(name), slot)
        v = jnp.sum(jnp.abs(v.astype(F32)).reshape(-1, 8, v.shape[1]), axis=0)
        total = size_v[at] + _total(v[:, c:c + BLK] for c in range(0, v.shape[1], BLK))
        size_v[at] = total
        return total

    def measure_all(name, ref, rows, first, cols, step):
        for c in range(first, first + cols, 256):
            for r in range(0, rows, step):
                yield [measure(name, r // step % ND, ref[r:r + step, c:c + 256])]

    def balance(source, target):
        def size(name):
            v = jnp.sum(size_v[list(SIZES).index(name)], axis=0)
            v = jnp.sum(jnp.sum(v, axis=0, keepdims=True), axis=1, keepdims=True)
            return jnp.clip(v / SIZES[name], 2.0 ** -30, 2.0 ** 30)
        ratio = jnp.broadcast_to(size(target) / size(source), (8, BLK))
        factor_v[list(SIZES).index(source)] = jnp.stack([ratio, 1 / ratio])

    def factors(source):
        return [jnp.concatenate([factor_v[list(SIZES).index(source), e]] * (BLK // 8))
                for e in range(2)]

    def store(ref, r, c, v):
        ref[r, c] = v

    def projections(b, half, y, c_done, z_done, b_scale=None):
        return _Pair(scratch, ND, ND, lambda i, j: xn_v[i, j], b,
                     lambda j, k: xn_v[ND * half + j, k], y, c_done, z_done, b_scale)

    def gate_up(half, ref, first):
        def up_done(i, j, v):
            h = v * h_v[ND * half + j, i]
            h_v[ND * half + j, i] = h
            measure("hidden", j, h)

        there, back = factors("gate")
        return projections(
            lambda j, k: wg_v[_block(j), _block(ND * (half + 1) + k)], half,
            lambda k, i: wu_v[_block(k), _block(i)],
            lambda i, k, v: store(ref, i, first + k, _sigmoid(v, back)), up_done, there)

    def project(k_v, qv_v, w_v):
        zero = lax.fori_loop(0, 2, lambda i, c: c * c + 2 * i, 2) - 18
        spare = pl.ds(pl.multiple_of(BLK + zero, 8), 8)

        def layernorm(tl, first, count):
            slabs = [(r, slice(r0, r0 + 8))
                     for r in range(first, first + count) for r0 in range(0, BLK, 8)]
            mean, var, scale = [], [], []
            for n in range(len(slabs) + 2 * LAG):
                tl.fence(x_v, 0, spare)
                done = []
                if n >= 2 * LAG:
                    k = n - 2 * LAG
                    xn = (x_v[slabs[k]].astype(F32) - mean[k]) * scale[k]
                    for g in range(ND):
                        xn_v[slabs[k][0], g, slabs[k][1]] = xn[:, BLK * g:BLK * (g + 1)]
                    measure("x", k % ND, jnp.broadcast_to(jnp.sqrt(var[k]) * scale[k], (8, BLK)))
                    done.append(xn)
                if LAG <= n < len(slabs) + LAG:
                    xc = x_v[slabs[n - LAG]].astype(F32) - mean[n - LAG]
                    var.append(jnp.mean(xc * xc, axis=-1, keepdims=True))
                    scale.append(lax.rsqrt(var[-1] + EPS))
                if n < len(slabs):
                    mean.append(jnp.mean(x_v[slabs[n]].astype(F32), axis=-1, keepdims=True))
                yield done

        def store_qv(half):
            def done(i, j, v):
                r = ND * half + j
                scale = jnp.where(i < ND, Q_SCALE, 1.0).astype(F32)
                qv_v[r // 4, i, :, _block(r % 4)] = (v * scale).T.astype(BF16)
            return done

        def w_qv(k, i):
            return w_v[_block(k), _block(i + i // ND * ND)]

        def x_copy(first, count):
            return x_hbm.at[first:first + count], x_v.at[first:first + count, :BLK]

        def w_copy(part, rows, cols):
            index = (slice(*rows), slice(DIM * part + cols[0], DIM * part + cols[1]))
            return wqkv_hbm.at[index], w_v.at[index]

        every = (0, DIM)
        copies = [
            pltpu.make_async_copy(*ends, in_sem.at[n]) for n, ends in enumerate([
                x_copy(0, 2), w_copy(1, (0, 256), every), w_copy(0, every, (0, 256)),
                x_copy(2, 2), w_copy(1, (256, 512), every), w_copy(0, every, (256, 512)),
                x_copy(4, 2), x_copy(6, 2), w_copy(1, (512, DIM), every),
                w_copy(0, every, (512, DIM)), x_copy(8, 8), w_copy(2, every, every),
                (wg_hbm.at[:, :DIM], wg_v.at[:, :DIM]), (wg_hbm.at[:, DIM:], wg_v.at[:, DIM:]),
                (wu_hbm, wu_v), (wd_hbm, wd_v)])
        ]

        def start(*numbers):
            for n in numbers:
                copies[n].start()

        def wait(*numbers):
            for n in numbers:
                copies[n].wait()

        start(*range(11))
        size_v[...] = jnp.zeros_like(size_v)
        pair = projections(lambda j, k: w_v[_block(j), _block(ND + k)], 0, w_qv,
                           lambda i, k, v: store(k_v, i, k, v.astype(BF16)), store_qv(0))
        wait(0)
        tl = timeline()
        _run(layernorm(tl, 0, 2))
        wait(1, 2)
        rows = [pair.row(tl, i, i < 4) for i in range(NR)]
        tl.add(8, rows[0])
        tl.add(4, rows[1], 1, 2)
        tl.emit()
        wait(3)
        _run(layernorm(tl, 2, 2))
        wait(4)
        tl.add(9, rows[0])
        tl.add(5, rows[1], 1, 2)
        tl.emit()
        wait(5, 6)
        tl.add(32 + 2 * LAG, layernorm(tl, 4, 2), 0, 1.8)
        tl.add(9, rows[2])
        tl.add(9, rows[3], 1, 2)
        tl.emit()
        wait(7, 8)
        start(11, 12)
        tl.add(32 + 2 * LAG, layernorm(tl, 6, 2), 0, 4.6)
        for i in range(4):
            tl.add(4 if i else 8, rows[i], i + 1 if i else 0, i + 2)
            tl.add(7 if i else 11, rows[i], 5 + i, 6 + i)
        tl.add(32, measure_all("qv", w_v, DIM, 0, 512, 64), 6, 8.8)
        tl.emit()
        wait(9, 10)
        tl.add(48 + 2 * LAG, layernorm(tl, ND, 3), 4, 7.9)
        tl.add(32, measure_all("qv", w_v, DIM, 512, 512, 64), 4, 7.9)
        for i in range(4, ND):
            tl.add(20, rows[i], i, i + 1)
        tl.emit()
        wait(11, 12)
        start(13)
        tl.add(80 + 2 * LAG, layernorm(tl, ND + 3, 5), ND, 14.8)
        tl.add(64, measure_all("qv", w_v, DIM, 2 * DIM, DIM, 64), ND, 13.5)
        tl.add(64, measure_all("gate0", wg_v, DIM, 0, DIM, 64), 13.5, 15.7)
        for i in range(ND, NR):
            tl.add(20, rows[i], i, i + 1)
        tl.emit()
        balance("gate0", "qv")
        wait(13)
        start(14, 15)

        there, back = factors("gate0")
        pair = projections(lambda j, k: wg_v[_block(j), _block(k)], 1, w_qv,
                           lambda i, k, v: store(h_v, i, k, _sigmoid(v, back)),
                           store_qv(1), there)
        pair.rows(timeline(), 0, NR)
        wait(14, 15)

    def attend(k_v, qv_v, s_v, max_v, ot_v, l_v):
        def position(step, u):
            return step // (ND // GB), step % (ND // GB) * GB + u

        def tile(tl, cur, nxt):
            for h in range(4 * GB):
                u, j = divmod(h, 4)
                head = slice(HEAD_DIM * j, HEAD_DIM * (j + 1))
                m = l = o = None
                if cur is not None:
                    _, g_cur = position(cur, u)
                    row_max = jnp.concatenate([max_v[h]] * (BLK // 8), axis=0)
                if nxt is not None:
                    t, g = position(nxt, u)
                    q = qv_v[t, g, head, :]
                    if j:
                        q = jnp.concatenate([jnp.zeros((head.start, TOK), BF16), q], axis=0)
                for r in range(NR):
                    if cur is not None:
                        s_old = s_v[h, r]
                    if nxt is not None:
                        s = _dot(k_v[r, g, :, :head.stop], q)
                        s_v[h, r] = tl.tie(tl.tie(tl.tie(s), 64), 96)
                        for r0 in range(0, BLK, 8):
                            m = s[r0:r0 + 8] if m is None else jnp.maximum(m, s[r0:r0 + 8])
                        if r == NR - 1:
                            max_v[h] = jnp.broadcast_to(
                                jnp.max(m, axis=0, keepdims=True), m.shape)
                    if cur is not None:
                        p = jnp.exp2(s_old - row_max)
                        for r0 in reversed(range(0, BLK, 8)):
                            l = p[r0:r0 + 8] if l is None else l + p[r0:r0 + 8]
                        pv = _dot(qv_v[r // 4, ND + g_cur, head, _block(r % 4)], p.astype(BF16))
                        o = pv if o is None else pv + o
                        if r == NR - 1:
                            l_v[h], ot_v[h] = l, o
                    yield []

        def normalize(step):
            for u in range(GB):
                t, g = position(step, u)
                for r in range(4):
                    cols = slice(BLK * r, BLK * (r + 1))
                    o = jnp.concatenate([
                        ot_v[h, :, cols] / jnp.sum(l_v[h, :, cols], axis=0, keepdims=True)
                        for h in range(4 * u, 4 * u + 4)], axis=0).T
                    o_v[4 * t + r, g] = o
                    yield [o]

        ot_v[...] = jnp.zeros_like(ot_v)
        l_v[...] = jnp.ones_like(l_v)
        tl = timeline()
        tl.add(80, measure_all("gate", wg_v, DIM, DIM, FFN - DIM, BLK), 0, 0.3)
        tl.add(112, measure_all("up", wu_v, DIM, 0, FFN, BLK), 0.3, 0.72)
        tl.add(64, measure_all("down", wd_v, 2 * DIM, 0, DIM, BLK), 0.72, 0.96)
        tl.add(4 * GB * NR, tile(tl, None, 0))
        tl.emit()
        balance("gate", "up")
        balance("down", "gate")

        def body(i, carry):
            tl = timeline()
            tl.add(4 * GB, normalize(jnp.maximum(i - 1, 0)), 0, 0.11)
            tl.add(4 * GB * NR, tile(tl, i, i + 1))
            tl.emit()
            return carry

        lax.fori_loop(0, STEPS - 1, body, 0)

        pair = gate_up(0, h_v, ND)
        tl = timeline()
        for i in range(NR):
            tl.add(20 if i else 36, pair.row(tl, i), i, i + 1)
        tl.add(4 * GB, normalize(STEPS - 2), 1, 2.5)
        last = tile(tl, STEPS - 1, None)
        after = (4, 6, 7, 10, 11, 12, 13, 14, 15, 16)
        for n in range(4 * GB * NR):
            when = 2 + n // len(after) + (after[n % len(after)] + 1) / 20
            tl.add(1, last, when, when)
        tl.add(4 * GB, normalize(STEPS - 1), 15, 15.8)
        tl.emit()

    def attention(k_v, qv_v):
        pl.run_scoped(lambda w_v: project(k_v, qv_v, w_v),
                      pltpu.VMEM((DIM, 3 * DIM), BF16))
        pl.run_scoped(lambda *refs: attend(k_v, qv_v, *refs),
                      pltpu.VMEM((4 * GB, NR, BLK, TOK), F32),
                      pltpu.VMEM((4 * GB, 8, TOK), F32),
                      pltpu.VMEM((4 * GB, HEAD_DIM, TOK), F32),
                      pltpu.VMEM((4 * GB, 8, TOK), F32))

    pl.run_scoped(attention,
                  pltpu.VMEM((NR, ND, BLK, BLK), BF16),
                  pltpu.VMEM((SEQ // TOK, 2 * ND, BLK, TOK), BF16))

    def glu(wo_v, out_v, *blocks):
        h2_v, y_v, *wide = map(_unpadded, blocks)

        wo_copy = pltpu.make_async_copy(wo_hbm, wo_v, in_sem.at[0])
        pair = gate_up(1, h2_v, 0)
        wo_copy.start()
        pair.rows(timeline(), 0, NR)
        balance("hidden", "x")
        wo_copy.wait()

        h_there, h_back = factors("hidden")
        w_there, w_back = factors("down")
        u_back, u_there = factors("gate")

        def gate_or_up(k, i):
            if isinstance(i, int):
                return wg_v[_block(k), _block(3 * ND + i)]
            return wu_v[_block(k), _block(2 * ND - 4 + i)].astype(F32) * u_there

        def hidden(i, j, v):
            if isinstance(i, int):
                h2_v[j, ND + i] = _sigmoid(v)
            else:
                h2_v[j, i - 4] = v * u_back * h2_v[j, i - 4]

        pair = _Pair(wide, NR, ND, lambda i, j: h_v[i, j] * h_there,
                     lambda j, k: wd_v[_block(j), _block(k)], lambda j, k: xn_v[j, k],
                     gate_or_up, lambda i, k, v: store(y_v, i, k, v * (h_back * w_back)),
                     hidden, w_there)
        pair.rows(timeline(), 0, 4)
        pair.loop(timeline, 4, 3, 4)

        def down(n, first, col, row, done):
            _Pair(scratch, n, n, lambda i, j: h2_v[i, first + j],
                  lambda j, k: wd_v[_block(NR + first + j), _block(col + k)],
                  lambda j, k: h2_v[row + j, first + k],
                  lambda k, i: wd_v[_block(NR + first + k), _block(i)],
                  lambda i, k, v: store(y_v, i, col + k, done(v)),
                  lambda i, j, v: store(y_v, row + j, i, done(v)),
                  c_init=lambda i, k: y_v[i, col + k],
                  z_init=lambda i, j: y_v[row + j, i]).rows(timeline(), 0, ND)

        def last_down(side, carry):
            down(4, ND, 4 * side, ND + 4 * side, lambda v: v)
            return carry

        lax.fori_loop(0, 2, last_down, 0)
        down(ND, 0, 0, ND, _silu)

        def finish(r, c, s):
            out = x_v[r, :BLK, _block(c)].astype(F32) + s * y_v[r, c]
            out_v[r, :, _block(c)] = out.astype(BF16)

        pair = _Pair(scratch, ND, ND, lambda i, j: o_v[i, j],
                     lambda j, k: wo_v[_block(j), _block(k)], lambda j, k: o_v[ND + j, k],
                     lambda k, i: wo_v[_block(k), _block(i)],
                     finish, lambda i, j, v: finish(ND + j, i, v))
        tl = timeline()
        done = []

        def write(*index):
            done.append(pltpu.make_async_copy(out_v.at[index], out_hbm.at[index], out_sem))
            done[-1].start()

        for first, stop in ((0, 5), (5, 7), (7, ND)):
            pair.rows(tl, first, stop - 1 - first)
            row = pair.row(tl, stop - 1)
            _run(zip(range(18), row) if stop == ND else row)
            write(slice(ND, NR), slice(0, BLK), slice(BLK * first, BLK * stop))
            _run(row)
            write(slice(first, stop))
        for c in done:
            c.wait()

    pl.run_scoped(glu,
                  pltpu.VMEM((DIM, DIM), BF16),
                  pltpu.VMEM((NR, BLK, DIM), BF16),
                  _blocks(NR, FFN // BLK - NR),
                  _blocks(NR, ND),
                  *_pair_scratch(NR))


@jax.jit
def pallas_recurrent_scan__softmax_full_mha__glu_gated_glu__prompt_kernel(
    A_x: jax.Array,
    A_wqkv: jax.Array,
    A_wo: jax.Array,
    B_x: jax.Array,
    B_w_gate: jax.Array,
    B_w_up: jax.Array,
    B_w_down: jax.Array,
):
    del B_x
    assert A_x.shape == (1, SEQ, DIM) and B_w_gate.shape == (DIM, FFN)
    out = pl.pallas_call(
        _kernel,
        out_shape=jax.ShapeDtypeStruct((NR, BLK, DIM), BF16),
        in_specs=[pl.BlockSpec(memory_space=pl.ANY)] * 6,
        out_specs=pl.BlockSpec(memory_space=pl.ANY),
        scratch_shapes=[
            pltpu.SemaphoreType.DMA((16,)),
            pltpu.SemaphoreType.DMA(()),
            pltpu.VMEM((NR, BLK + 16, DIM), BF16),
            pltpu.VMEM((DIM, FFN), BF16),
            pltpu.VMEM((DIM, FFN), BF16),
            pltpu.VMEM((FFN, DIM), BF16),
            pltpu.VMEM((len(SIZES), ND, 8, BLK), F32),
            pltpu.VMEM((8, 2, 8, BLK), F32),
            _blocks(NR, ND),
            _blocks(NR, ND),
            _blocks(NR, NR),
            *_pair_scratch(ND),
        ],
        compiler_params=pltpu.CompilerParams(vmem_limit_bytes=127 * 2**20),
        name="mha_glu",
    )(A_x.reshape(NR, BLK, DIM), A_wqkv, A_wo, B_w_gate, B_w_up, B_w_down)
    return out.reshape(A_x.shape)
```
